```python
import os as _os
_os.environ.setdefault("JAX_PLATFORMS", "cpu")
import jax
import jax.numpy as jnp

def _softmax(x, axis=-1):
    return jax.nn.softmax(x, axis=axis)
def _gelu(x):
    return jax.nn.gelu(x, approximate=True)
def _silu(x):
    return jax.nn.silu(x)
def _sigmoid(x):
    return jax.nn.sigmoid(x)
def _layernorm(x, axis=-1, eps=1e-5):
    m = jnp.mean(x, axis=axis, keepdims=True)
    v = jnp.var(x, axis=axis, keepdims=True)
    return (x - m) / jnp.sqrt(v + eps)
def _scatter_add(tgt, idx, src, axis=0):
    return tgt.at[idx].add(src)
def _segment_sum(src, seg, n):
    return jax.ops.segment_sum(src, seg, n)
class _Rng:
    def __init__(self, key):
        self._k = key
    def _next(self):
        self._k, sub = jax.random.split(self._k)
        return sub
    def normal(self, shape):
        return jax.random.normal(self._next(), shape, dtype=jnp.bfloat16)
    def randint(self, lo, hi, shape):
        return jax.random.randint(self._next(), shape, lo, hi, dtype=jnp.int32)
    def uniform(self, shape, lo=0.0, hi=1.0):
        return jax.random.uniform(self._next(), shape, jnp.bfloat16, lo, hi)
    def permutation(self, n):
        return jax.random.permutation(self._next(), n)


kernel_name = 'concat_heads__mha_block_cached__gqa_block_cached__decode'

def setup_inputs():
    _rng = _Rng(jax.random.key(int.from_bytes(__import__("os").urandom(4), "little")))
    _w = (lambda a: (lambda t: t.astype(jnp.bfloat16) if jnp.issubdtype(t.dtype, jnp.floating) else t)(jnp.asarray(a)))
    def _A_setup():
        B, Sq, D = 1, 1, 512
        H, Sk, Dh = 32, 4096, 128
        return {
            "x": _w((lambda *s: _rng.normal(s) * 0.8)(B, Sq, D)),
            "k_cache": _w((lambda *s: _rng.normal(s) * 0.8)(B, H, Sk, Dh)),
            "v_cache": _w((lambda *s: _rng.normal(s) * 0.05)(B, H, Sk, Dh)),
            "wq": _w((lambda *s: _rng.normal(s) * 0.8)(D, H * Dh) * (D ** -0.5)),
            "wo": _w((lambda *s: _rng.normal(s) * 0.05)(H * Dh, D) * ((H * Dh) ** -0.5)),
        }
    _A_in = _A_setup()

    def _B_setup():
        B, Sq, D = 1, 1, 512
        Hq, Hkv, Sk, Dh = 32, 32, 4096, 128
        assert Hq % Hkv == 0, (Hq, Hkv)
        return {
            "x": _w((lambda *s: _rng.normal(s) * 0.8)(B, Sq, D)),
            "k_cache": _w((lambda *s: _rng.normal(s) * 0.8)(B, Hkv, Sk, Dh)),
            "v_cache": _w((lambda *s: _rng.normal(s) * 0.05)(B, Hkv, Sk, Dh)),
            "wq": _w((lambda *s: _rng.normal(s) * 0.8)(D, Hq * Dh) * (D ** -0.5)),
            "wo": _w((lambda *s: _rng.normal(s) * 0.05)(Hq * Dh, D) * ((Hq * Dh) ** -0.5)),
        }
    _B_in = _B_setup()

    return {
        "A_x": _A_in["x"],
        "A_k_cache": _A_in["k_cache"],
        "A_v_cache": _A_in["v_cache"],
        "A_wq": _A_in["wq"],
        "A_wo": _A_in["wo"],
        "B_x": _B_in["x"],
        "B_k_cache": _B_in["k_cache"],
        "B_v_cache": _B_in["v_cache"],
        "B_wq": _B_in["wq"],
        "B_wo": _B_in["wo"],
    }

def reference(A_x, A_k_cache, A_v_cache, A_wq, A_wo, B_x, B_k_cache, B_v_cache, B_wq, B_wo):
    def _A_ref(x, k_cache, v_cache, wq, wo):
        B, Sq, D = x.shape
        H, Dh = 32, 128
        q = (lambda x, *d: x.transpose(*d))((x @ wq).reshape(B, Sq, H, Dh), 0, 2, 1, 3)
        scores = jnp.einsum("bhqd,bhkd->bhqk", q, k_cache) * (Dh ** -0.5)
        p = _softmax(scores, axis=-1)
        o = jnp.einsum("bhqk,bhkd->bhqd", p, v_cache)
        return (lambda x, *d: x.transpose(*d))(o, 0, 2, 1, 3).reshape(B, Sq, H * Dh) @ wo

    def _B_ref(x, k_cache, v_cache, wq, wo):
        B, Sq, D = x.shape
        Hq, Dh = 32, 128
        Hkv = k_cache.shape[1]
        rep = Hq // Hkv
        q = (lambda x, *d: x.transpose(*d))((x @ wq).reshape(B, Sq, Hq, Dh), 0, 2, 1, 3)
        k = jnp.repeat(k_cache, rep, axis=1)
        v = jnp.repeat(v_cache, rep, axis=1)
        scores = jnp.einsum("bhqd,bhkd->bhqk", q, k) * (Dh ** -0.5)
        p = _softmax(scores, axis=-1)
        o = jnp.einsum("bhqk,bhkd->bhqd", p, v)
        return (lambda x, *d: x.transpose(*d))(o, 0, 2, 1, 3).reshape(B, Sq, Hq * Dh) @ wo

    a = _A_ref(A_x, A_k_cache, A_v_cache, A_wq, A_wo)
    b = _B_ref(B_x, B_k_cache, B_v_cache, B_wq, B_wo)
    return jnp.concatenate([a, b], axis=-1)
```

```python
import functools
import jax
import jax.numpy as jnp
from jax import lax
from jax.experimental import pallas as pl
from jax.experimental.pallas import tpu as pltpu

D, H, SK, DH = 512, 32, 4096, 128
HG = 8
NG = H // HG


def make(nh=2, rr=64, T=256, lag=4, nslot=8, nobc=True, compute=True):
    NT = SK // T
    NKV = NG * NT
    NW = 8
    scale = DH ** -0.5
    assert lag <= nslot - 1 and lag <= NW and nslot & (nslot - 1) == 0

    def body(ax, ak, av, awq, awo, bx, bk, bv, bwq, bwo, o_ref,
             xbuf, wqbuf, wobuf, ring, q_ref, s_ref, p_ref, acc_ref,
             xsem, wqsem, wosem, rsem):
        def start_wq(i):
            c0 = pl.multiple_of(i * 512, 512)
            for r in range(16):
                for p, w in enumerate((awq, bwq)):
                    pltpu.make_async_copy(
                        w.at[:, pl.ds(r * 8, 8), pl.ds(c0, 512)],
                        wqbuf.at[i, p, :, pl.ds(r * 8, 8), :], wqsem.at[i]).start(priority=p)

        def start_wo(i):
            for r in range(16):
                for p, w in enumerate((awo, bwo)):
                    pltpu.make_async_copy(
                        w.at[:, pl.ds(pl.multiple_of(i * 128 + r * 8, 8), 8), :],
                        wobuf.at[i, p, :, pl.ds(r * 8, 8), :], wosem.at[i]).start(priority=p)

        def start_kv(srcs, i):
            slot = i & (nslot - 1)
            h0 = (i // NT) * HG
            t0 = (i & (NT - 1)) * T
            for r in range(T // rr):
                for hb in range(HG // nh):
                    for p, src in enumerate(srcs):
                        pltpu.make_async_copy(
                            src.at[pl.ds(h0 + hb * nh, nh), pl.ds(pl.multiple_of(t0 + r * rr, rr), rr), :],
                            ring.at[slot, p, pl.ds(hb * nh, nh), pl.ds(r * rr, rr), :],
                            rsem.at[slot]).start(priority=p)

        def wait(buf, sem):
            pltpu.make_async_copy(buf, buf, sem).wait()

        def issue(i, n, cur, nxt):
            @pl.when(i + lag < n)
            def _():
                cur(i + lag)
            if nxt is not None:
                @pl.when(i + lag >= n)
                def _():
                    nxt(i + lag - n)

        start_k = functools.partial(start_kv, (ak, bk))
        start_v = functools.partial(start_kv, (av, bv))

        start_wq(0)
        xa = pltpu.make_async_copy(ax, xbuf.at[0], xsem.at[0])
        xb = pltpu.make_async_copy(bx, xbuf.at[1], xsem.at[1])
        xa.start()
        xb.start(priority=1)
        lax.fori_loop(1, lag, lambda i, _: start_wq(i), None)
        xa.wait()
        xb.wait()

        row = lax.broadcasted_iota(jnp.int32, (HG, 1), 0)

        def wq_step(i, _):
            issue(i, NW, start_wq, start_k)
            wait(wqbuf.at[i], wqsem.at[i])
            if not compute:
                return
            for p in range(2):
                x = jnp.broadcast_to(xbuf[p, 0], (HG, D))
                w = wqbuf[i, p].reshape(D, 512)
                q = jnp.dot(x, w, preferred_element_type=jnp.float32)
                for j in range(4):
                    q_ref[p, pl.ds(i * 4 + j, 1), :] = q[0:1, j * DH:(j + 1) * DH]
        lax.fori_loop(0, NW, wq_step, None)

        def k_group(g, _):
            def k_step(t, _):
                i = g * NT + t
                issue(i, NKV, start_k, start_v)
                slot = i & (nslot - 1)
                wait(ring.at[slot], rsem.at[slot])
                if not compute:
                    return
                for p in range(2):
                    q = q_ref[p, pl.ds(pl.multiple_of(g * HG, HG), HG), :].astype(jnp.bfloat16)
                    s = None
                    for h in range(HG):
                        sh = lax.dot_general(q, ring[slot, p, h], (((1,), (1,)), ((), ())),
                                             preferred_element_type=jnp.float32)
                        s = sh if s is None else jnp.where(row == h, sh, s)
                    s_ref[p, t] = s * scale
            lax.fori_loop(0, NT, k_step, None)
            if not compute:
                return
            for p in range(2):
                s = s_ref[p]
                m = jnp.max(jnp.max(s, axis=0), axis=-1, keepdims=True)
                e = jnp.exp(s - m)
                l = jnp.sum(jnp.sum(e, axis=0), axis=-1, keepdims=True)
                p_ref[p, g] = e * (1.0 / l)
        lax.fori_loop(0, NG, k_group, None)

        def v_group(g, _):
            def v_step(t, acc):
                i = g * NT + t
                issue(i, NKV, start_v, start_wo)
                slot = i & (nslot - 1)
                wait(ring.at[slot], rsem.at[slot])
                if not compute:
                    return acc
                out = []
                for p in range(2):
                    pr = p_ref[p, g, t].astype(jnp.bfloat16)
                    o = None
                    for h in range(HG):
                        oh = jnp.dot(pr, ring[slot, p, h], preferred_element_type=jnp.float32)
                        o = oh if o is None else jnp.where(row == h, oh, o)
                    out.append(acc[p] + o)
                return tuple(out)
            z = jnp.zeros((HG, DH), jnp.float32)
            acc = lax.fori_loop(0, NT, v_step, (z, z))
            for p in range(2):
                acc_ref[p, g] = acc[p]
        lax.fori_loop(0, NG, v_group, None)

        def wo_step(i, acc):
            issue(i, NW, start_wo, None)
            wait(wobuf.at[i], wosem.at[i])
            if not compute:
                return acc
            out = []
            for p in range(2):
                o = jnp.concatenate(
                    [jnp.broadcast_to(acc_ref[p, g, pl.ds(i, 1), :], (HG, DH)) for g in range(NG)],
                    axis=-1).astype(jnp.bfloat16)
                w = wobuf[i, p].reshape(NG * DH, D)
                out.append(acc[p] + jnp.dot(o, w, preferred_element_type=jnp.float32))
            return tuple(out)
        z = jnp.zeros((HG, D), jnp.float32)
        acc = lax.fori_loop(0, NW, wo_step, (z, z))
        o_ref[0] = jnp.concatenate([acc[0][0:1], acc[1][0:1]], axis=-1).astype(o_ref.dtype)

    def fn(A_x, A_k, A_v, A_wq, A_wo, B_x, B_k, B_v, B_wq, B_wo):
        hbm = pl.BlockSpec(memory_space=pltpu.HBM)
        kv = lambda a: a.reshape(H, SK, DH)
        wq = lambda a: a.reshape(4, D // 4, H * DH)
        wo = lambda a: a.reshape(NG, HG * DH, D)
        bf = jnp.bfloat16
        return pl.pallas_call(
            body,
            out_shape=jax.ShapeDtypeStruct((1, 1, 2 * D), bf),
            in_specs=[hbm] * 10,
            out_specs=pl.BlockSpec(memory_space=pltpu.VMEM),
            scratch_shapes=[
                pltpu.VMEM((2, 1, 1, D), bf),
                pltpu.VMEM((NW, 2, 4, 128, 512), bf),
                pltpu.VMEM((NW, 2, NG, DH, D), bf),
                pltpu.VMEM((nslot, 2, HG, T, DH), bf),
                pltpu.VMEM((2, H, DH), jnp.float32),
                pltpu.VMEM((2, NT, HG, T), jnp.float32),
                pltpu.VMEM((2, NG, NT, HG, T), jnp.float32),
                pltpu.VMEM((2, NG, HG, DH), jnp.float32),
                pltpu.SemaphoreType.DMA((2,)),
                pltpu.SemaphoreType.DMA((NW,)),
                pltpu.SemaphoreType.DMA((NW,)),
                pltpu.SemaphoreType.DMA((nslot,)),
            ],
            compiler_params=pltpu.CompilerParams(
                vmem_limit_bytes=100 * 2**20, disable_bounds_checks=nobc),
        )(A_x, kv(A_k), kv(A_v), wq(A_wq), wo(A_wo), B_x, kv(B_k), kv(B_v), wq(B_wq), wo(B_wo))
    return fn


@jax.jit
def pallas_concat_heads__mha_block_cached__gqa_block_cached__decode_kernel(
        A_x, A_k_cache, A_v_cache, A_wq, A_wo, B_x, B_k_cache, B_v_cache, B_wq, B_wo):
    return make()(A_x, A_k_cache, A_v_cache, A_wq, A_wo, B_x, B_k_cache, B_v_cache, B_wq, B_wo)
```

```python
import functools
import jax
import jax.numpy as jnp
from jax import lax
from jax.experimental import pallas as pl
from jax.experimental.pallas import tpu as pltpu

D, H, SK, DH = 512, 32, 4096, 128
HG = 8
NG = H // HG


def make(nh=2, rr=64, T=256, lag=4, nslot=8, nobc=False, nosc=False, skew=0, wq16=True, tail=4,
         hb_order=None, wnh=2, shift=0):
    NT = SK // T
    NKV = NG * NT
    NW = 8
    scale = DH ** -0.5
    hb_order = hb_order or tuple(range(HG // nh))
    assert lag <= nslot - 1 and lag < NW and nslot & (nslot - 1) == 0

    def body(ax, ak, av, awq, awo, bx, bk, bv, bwq, bwo, o_ref,
             xbuf, wqbuf, wobuf, ring, s_ref, p_ref, acc_ref, tsem):
        def wait(buf, sem):
            pltpu.make_async_copy(buf, buf, sem).wait()

        def key_block(p, t):
            return (t + skew) & (NT - 1) if p and skew else t

        def main(wqsem, rsem):
            wc = 2048 // wnh
            wr = 32 // wnh

            def start_wq(i):
                stripes = (i, i + 8) if wq16 else (2 * i, 2 * i + 1)
                order = ([(c, r) for c in range(H * DH // wc) for r in stripes] if wq16 else
                         [(c, r) for r in stripes for c in range(H * DH // wc)])
                for c, r in order:
                    r0 = pl.multiple_of(r * 8, 8)
                    for a in range(4 // wnh):
                        for p, w in enumerate((awq, bwq)):
                            idx = (pl.ds(wnh * a, wnh), pl.ds(r0, 8), pl.ds(c * wc, wc))
                            pltpu.make_async_copy(w.at[idx], wqbuf.at[(p,) + idx], wqsem).start(priority=p)

            def start_wo(i):
                slot = i & (nslot - 1)
                for r in range(DH // wr):
                    for a in range(NG // wnh):
                        for p, w in enumerate((awo, bwo)):
                            pltpu.make_async_copy(
                                w.at[pl.ds(wnh * a, wnh), pl.ds(pl.multiple_of(i * DH + r * wr, wr), wr), :],
                                wobuf.at[i, pl.ds(wnh * a, wnh), p, pl.ds(r * wr, wr), :],
                                rsem.at[slot]).start(priority=p)

            def start_wo_tail():
                i = NW - 1
                per = NG // tail
                for u in range(tail):
                    for r in range(DH // 32):
                        for g in range(u * per, (u + 1) * per):
                            for p, w in enumerate((awo, bwo)):
                                pltpu.make_async_copy(
                                    w.at[g, pl.ds(i * DH + r * 32, 32), :],
                                    wobuf.at[i, g, p, pl.ds(r * 32, 32), :],
                                    tsem.at[u]).start(priority=p)

            def start_kv(srcs, i):
                slot = i & (nslot - 1)
                h0 = (i // NT) * HG
                for r in range(T // rr):
                    for hb in hb_order:
                        for p, src in enumerate(srcs):
                            t0 = key_block(p, i & (NT - 1)) * T
                            pltpu.make_async_copy(
                                src.at[pl.ds(h0 + hb * nh, nh), pl.ds(pl.multiple_of(t0 + r * rr, rr), rr), :],
                                ring.at[slot, p, pl.ds(hb * nh, nh), pl.ds(r * rr, rr), :],
                                rsem.at[slot]).start(priority=p)

            def issue(i, n, cur, nxt):
                @pl.when(i + lag < n)
                def _():
                    cur(i + lag)

                @pl.when(i + lag >= n)
                def _():
                    nxt(i + lag - n)

            start_k = functools.partial(start_kv, (ak, bk))
            start_v = functools.partial(start_kv, (av, bv))

            lax.fori_loop(0, 8, lambda i, _: start_wq(i), None)
            xa = pltpu.async_copy(ax, xbuf.at[0], wqsem)
            xb = pltpu.async_copy(bx, xbuf.at[1], wqsem, priority=1)
            lax.fori_loop(0, lag, lambda i, _: start_k(i), None)
            xa.wait()
            xb.wait()
            wait(wqbuf, wqsem)

            row = lax.broadcasted_iota(jnp.int32, (HG, 1), 0)

            def k_group(g, _):
                qs = []
                for p in range(2):
                    x = jnp.broadcast_to(xbuf[p, 0], (HG, D))
                    w = wqbuf[p, :, :, pl.ds(pl.multiple_of(g * HG * DH, HG * DH), HG * DH)]
                    qf = jnp.dot(x, w.reshape(D, HG * DH), preferred_element_type=jnp.float32)
                    q = qf[:, :DH]
                    for h in range(1, HG):
                        q = jnp.where(row == h, qf[:, h * DH:(h + 1) * DH], q)
                    qs.append(q.astype(jnp.bfloat16))

                def k_step(t, _):
                    i = g * NT + t
                    issue(i, NKV, start_k, start_v)
                    slot = i & (nslot - 1)
                    wait(ring.at[slot], rsem.at[slot])
                    for p in range(2):
                        s = None
                        for h in range(HG):
                            sh = lax.dot_general(qs[p], ring[slot, p, h], (((1,), (1,)), ((), ())),
                                                 preferred_element_type=jnp.float32)
                            s = sh if s is None else jnp.where(row == h, sh, s)
                        s_ref[p, t] = s * scale
                lax.fori_loop(0, NT, k_step, None)
                for p in range(2):
                    s = s_ref[p]
                    m = jnp.max(jnp.max(s, axis=0), axis=-1, keepdims=True)
                    e = jnp.exp(s - m)
                    l = jnp.sum(jnp.sum(e, axis=0), axis=-1, keepdims=True)
                    p_ref[p, g] = e * (1.0 / l)
            lax.fori_loop(0, NG, k_group, None)

            def v_group(g, _):
                def v_step(t, acc):
                    i = g * NT + t
                    issue(i, NKV, start_v, start_wo)
                    slot = i & (nslot - 1)
                    wait(ring.at[slot], rsem.at[slot])
                    out = []
                    for p in range(2):
                        pr = p_ref[p, g, t].astype(jnp.bfloat16)
                        o = None
                        for h in range(HG):
                            oh = jnp.dot(pr, ring[slot, p, h], preferred_element_type=jnp.float32)
                            o = oh if o is None else jnp.where(row == h, oh, o)
                        out.append(acc[p] + o)
                    return tuple(out)
                z = jnp.zeros((HG, DH), jnp.float32)
                acc = lax.fori_loop(0, NT, v_step, (z, z))
                for p in range(2):
                    acc_ref[p, g] = acc[p]
            lax.fori_loop(0, NG, v_group, None)

            def wo_step(i, acc):
                @pl.when(i + lag < NW - 1)
                def _():
                    start_wo(i + lag)

                @pl.when(i + lag == NW - 1)
                def _():
                    start_wo_tail()
                wait(wobuf.at[i], rsem.at[i & (nslot - 1)])
                return project(acc, i, range(NG))
            z = jnp.zeros((HG, D), jnp.float32)
            return lax.fori_loop(0, NW - 1, wo_step, (z, z))

        def project(acc, i, groups):
            out = []
            for p in range(2):
                a = acc[p]
                for g in groups:
                    o = jnp.broadcast_to(acc_ref[p, g, pl.ds(i, 1), :], (HG, DH)).astype(jnp.bfloat16)
                    a = a + jnp.dot(o, wobuf[i, g, p], preferred_element_type=jnp.float32)
                out.append(a)
            return tuple(out)

        acc = pl.run_scoped(main, pltpu.SemaphoreType.DMA(()), pltpu.SemaphoreType.DMA((nslot,)))
        per = NG // tail
        for u in range(tail):
            wait(wobuf.at[NW - 1, pl.ds(u * per, per)], tsem.at[u])
            acc = project(acc, NW - 1, range(u * per, (u + 1) * per))
        o_ref[0] = jnp.concatenate([acc[0][0:1], acc[1][0:1]], axis=-1).astype(o_ref.dtype)

    def fn(A_x, A_k, A_v, A_wq, A_wo, B_x, B_k, B_v, B_wq, B_wo):
        hbm = pl.BlockSpec(memory_space=pltpu.HBM)
        kv = lambda a: a.reshape(H, SK, DH)
        wq = lambda a: a.reshape(4, D // 4, H * DH)
        wo = lambda a: a.reshape(NG, HG * DH, D)
        bf = jnp.bfloat16
        return pl.pallas_call(
            body,
            out_shape=jax.ShapeDtypeStruct((1, 1, 2 * D), bf),
            in_specs=[hbm] * 10,
            out_specs=pl.BlockSpec(memory_space=pltpu.VMEM),
            scratch_shapes=[
                pltpu.VMEM((2, 1, 1, D), bf),
                pltpu.VMEM((2, 4, D // 4, H * DH), bf),
                pltpu.VMEM((NW, NG, 2, DH, D), bf),
                pltpu.VMEM((nslot, 2, HG, T, DH), bf),
                pltpu.VMEM((2, NT, HG, T), jnp.float32),
                pltpu.VMEM((2, NG, NT, HG, T), jnp.float32),
                pltpu.VMEM((2, NG, HG, DH), jnp.float32),
                pltpu.SemaphoreType.DMA((tail,)),
            ],
            compiler_params=pltpu.CompilerParams(
                vmem_limit_bytes=100 * 2**20, disable_bounds_checks=nobc, disable_semaphore_checks=nosc),
        )(A_x, kv(A_k), kv(A_v), wq(A_wq), wo(A_wo), B_x, kv(B_k), kv(B_v), wq(B_wq), wo(B_wo))
    return fn


@jax.jit
def pallas_concat_heads__mha_block_cached__gqa_block_cached__decode_kernel(
        A_x, A_k_cache, A_v_cache, A_wq, A_wo, B_x, B_k_cache, B_v_cache, B_wq, B_wo):
    return make(1, 128, wnh=1, tail=2)(A_x, A_k_cache, A_v_cache, A_wq, A_wo, B_x, B_k_cache, B_v_cache, B_wq, B_wo)
```

```python
import functools

import jax
import jax.numpy as jnp
from jax import lax
import jax.experimental.pallas as pl
import jax.experimental.pallas.tpu as pltpu

D, H, SK, DH = 512, 32, 4096, 128
HG = 8
NG = H // HG
T = 256
NT = SK // T
NKV = NG * NT
NSLOT = 4
LAG = NSLOT - 1
NE = 6
WO_TAIL = ((6, 0, 4), (7, 0, 2), (7, 2, 2))
SCALE = DH ** -0.5


def _wait(buf, sem):
    pltpu.make_async_copy(buf, buf, sem).wait()


def _per_head(f):
    row = lax.broadcasted_iota(jnp.int32, (HG, 1), 0)
    out = f(0)
    for j in range(1, HG):
        out = jnp.where(row == j, f(j), out)
    return out


def _kernel(ax, ak, av, awq, awo, bx, bk, bv, bwq, bwo, out_hbm,
            xbuf, wqbuf, wobuf, ring, s_ref, p_ref, o_ref, outbuf, out_sem):

    def start_wq(u, c, a, sem):
        idx = (pl.ds(a, 2), pl.ds(pl.multiple_of(u * 8, 8), 8), pl.ds(c * 1024, 1024))
        for p, w in enumerate((awq, bwq)):
            pltpu.async_copy(w.at[idx], wqbuf.at[(p,) + idx], sem, priority=p)

    def start_wo(i, g, r, sem):
        for p, w in enumerate((awo, bwo)):
            pltpu.async_copy(w.at[pl.ds(g, 2), i, pl.ds(r, 16), :],
                             wobuf.at[i, pl.ds(g, 2), p, pl.ds(r, 16), :], sem, priority=p)

    def project(out, i, groups):
        res = []
        for p in range(2):
            acc = out[p]
            for g in groups:
                o = jnp.broadcast_to(o_ref[p, g, pl.ds(i, 1), :], (HG, DH)).astype(jnp.bfloat16)
                acc = acc + jnp.dot(o, wobuf[i, g, p], preferred_element_type=jnp.float32)
            res.append(acc)
        return tuple(res)

    def main(ring_sems, tail_sems):
        def start_kv(srcs, step):
            slot = step & (NSLOT - 1)
            h0 = (step // NT) * HG
            t0 = (step & (NT - 1)) * T
            for r in range(0, T, 64):
                for j in range(0, HG, 2):
                    for p, src in enumerate(srcs):
                        pltpu.async_copy(
                            src.at[pl.ds(h0 + j, 2), pl.ds(pl.multiple_of(t0 + r, 64), 64), :],
                            ring.at[slot, p, pl.ds(j, 2), pl.ds(r, 64), :],
                            ring_sems.at[slot], priority=p)

        def start_wo_tail(i):
            for u, (head, g0, n) in enumerate(WO_TAIL):
                if head == i:
                    for r in range(0, DH, 16):
                        for g in range(g0, g0 + n, 2):
                            start_wo(i, g, r, tail_sems.at[u])

        start_k = functools.partial(start_kv, (ak, bk))
        start_v = functools.partial(start_kv, (av, bv))

        def prologue(sems):
            def start_weights(with_wo, u, _):
                for c in range(4):
                    for a in (0, 2):
                        start_wq(u, c, a, sems.at[0])
                    if with_wo:
                        for g in (0, 2):
                            start_wo(u >> 1, g, pl.multiple_of((u & 1) * 64 + c * 16, 16), sems.at[1])

            lax.fori_loop(0, 2 * NE, functools.partial(start_weights, True), None)
            lax.fori_loop(2 * NE, D // 4 // 8, functools.partial(start_weights, False), None)
            xa = pltpu.async_copy(ax, xbuf.at[0], sems.at[2], priority=0)
            xb = pltpu.async_copy(bx, xbuf.at[1], sems.at[3], priority=1)
            lax.fori_loop(0, LAG, lambda step, _: start_k(step), None)
            _wait(wqbuf, sems.at[0])
            _wait(wobuf.at[pl.ds(0, NE)], sems.at[1])
            xa.wait()
            xb.wait()

        pl.run_scoped(prologue, pltpu.SemaphoreType.DMA((4,)))

        def k_group(g, _):
            qs = []
            for p in range(2):
                x = jnp.broadcast_to(xbuf[p, 0], (HG, D))
                w = wqbuf[p, :, :, pl.ds(pl.multiple_of(g * HG * DH, HG * DH), HG * DH)]
                q = jnp.dot(x, w.reshape(D, HG * DH), preferred_element_type=jnp.float32)
                qs.append(_per_head(lambda j: q[:, j * DH:(j + 1) * DH]).astype(jnp.bfloat16))

            def k_step(t, _):
                step = g * NT + t
                pl.when(step + LAG < NKV)(lambda: start_k(step + LAG))
                pl.when(step + LAG >= NKV)(lambda: start_v(step + LAG - NKV))
                slot = step & (NSLOT - 1)
                _wait(ring.at[slot], ring_sems.at[slot])
                for p in range(2):
                    s_ref[p, t] = SCALE * _per_head(lambda j: lax.dot_general(
                        qs[p], ring[slot, p, j], (((1,), (1,)), ((), ())),
                        preferred_element_type=jnp.float32))

            lax.fori_loop(0, NT, k_step, None)
            for p in range(2):
                s = s_ref[p]
                m = jnp.max(jnp.max(s, axis=0), axis=-1, keepdims=True)
                e = jnp.exp(s - m)
                p_ref[p, g] = e / jnp.sum(jnp.sum(e, axis=0), axis=-1, keepdims=True)

        lax.fori_loop(0, NG, k_group, None)

        def v_group(g, out):
            def v_step(t, o):
                step = g * NT + t
                pl.when(step + LAG < NKV)(lambda: start_v(step + LAG))
                for k in range(HG - NE):
                    pl.when(step + LAG == NKV + k)(functools.partial(start_wo_tail, NE + k))
                slot = step & (NSLOT - 1)
                _wait(ring.at[slot], ring_sems.at[slot])
                res = []
                for p in range(2):
                    probs = p_ref[p, g, t].astype(jnp.bfloat16)
                    res.append(o[p] + _per_head(lambda j: jnp.dot(
                        probs, ring[slot, p, j], preferred_element_type=jnp.float32)))
                return tuple(res)

            zero = jnp.zeros((HG, DH), jnp.float32)
            o = lax.fori_loop(0, NT, v_step, (zero, zero))
            for p in range(2):
                o_ref[p, g] = o[p]
            for i in range(NE):
                out = project(out, i, (g,))
            return out

        zero = jnp.zeros((HG, D), jnp.float32)
        out = lax.fori_loop(0, NG, v_group, (zero, zero))
        for u, (i, g0, n) in enumerate(WO_TAIL):
            _wait(wobuf.at[i, pl.ds(g0, n)], tail_sems.at[u])
            out = project(out, i, range(g0, g0 + n))
        outbuf[0] = jnp.concatenate([out[0][0:1], out[1][0:1]], axis=-1).astype(outbuf.dtype)
        pltpu.make_async_copy(outbuf, out_hbm, out_sem).start()

    pl.run_scoped(main, pltpu.SemaphoreType.DMA((NSLOT,)), pltpu.SemaphoreType.DMA((len(WO_TAIL),)))
    pltpu.make_async_copy(outbuf, out_hbm, out_sem).wait()


@jax.jit
def pallas_concat_heads__mha_block_cached__gqa_block_cached__decode_kernel(
    A_x: jax.Array,
    A_k_cache: jax.Array,
    A_v_cache: jax.Array,
    A_wq: jax.Array,
    A_wo: jax.Array,
    B_x: jax.Array,
    B_k_cache: jax.Array,
    B_v_cache: jax.Array,
    B_wq: jax.Array,
    B_wo: jax.Array,
):
    dtype = A_x.dtype
    hbm = pl.BlockSpec(memory_space=pltpu.HBM)

    def operands(x, k, v, wq, wo):
        return (x, k.reshape(H, SK, DH), v.reshape(H, SK, DH),
                wq.reshape(4, D // 4, H * DH), wo.reshape(NG, HG, DH, D))

    return pl.pallas_call(
        _kernel,
        out_shape=jax.ShapeDtypeStruct((1, 1, 2 * D), dtype),
        in_specs=[hbm] * 10,
        out_specs=hbm,
        scratch_shapes=[
            pltpu.VMEM((2, 1, 1, D), dtype),
            pltpu.VMEM((2, 4, D // 4, H * DH), dtype),
            pltpu.VMEM((HG, NG, 2, DH, D), dtype),
            pltpu.VMEM((NSLOT, 2, HG, T, DH), dtype),
            pltpu.VMEM((2, NT, HG, T), jnp.float32),
            pltpu.VMEM((2, NG, NT, HG, T), jnp.float32),
            pltpu.VMEM((2, NG, HG, DH), jnp.float32),
            pltpu.VMEM((1, 1, 2 * D), dtype),
            pltpu.SemaphoreType.DMA(()),
        ],
        compiler_params=pltpu.CompilerParams(vmem_limit_bytes=32 * 2**20),
    )(*operands(A_x, A_k_cache, A_v_cache, A_wq, A_wo),
      *operands(B_x, B_k_cache, B_v_cache, B_wq, B_wo))
```
